```python
import os as _os
_os.environ.setdefault("JAX_PLATFORMS", "cpu")
import jax
import jax.numpy as jnp

def _softmax(x, axis=-1):
    return jax.nn.softmax(x, axis=axis)
def _gelu(x):
    return jax.nn.gelu(x, approximate=True)
def _silu(x):
    return jax.nn.silu(x)
def _sigmoid(x):
    return jax.nn.sigmoid(x)
def _layernorm(x, axis=-1, eps=1e-5):
    m = jnp.mean(x, axis=axis, keepdims=True)
    v = jnp.var(x, axis=axis, keepdims=True)
    return (x - m) / jnp.sqrt(v + eps)
def _scatter_add(tgt, idx, src, axis=0):
    return tgt.at[idx].add(src)
def _segment_sum(src, seg, n):
    return jax.ops.segment_sum(src, seg, n)
class _Rng:
    def __init__(self, key):
        self._k = key
    def _next(self):
        self._k, sub = jax.random.split(self._k)
        return sub
    def normal(self, shape):
        return jax.random.normal(self._next(), shape, dtype=jnp.bfloat16)
    def randint(self, lo, hi, shape):
        return jax.random.randint(self._next(), shape, lo, hi, dtype=jnp.int32)
    def uniform(self, shape, lo=0.0, hi=1.0):
        return jax.random.uniform(self._next(), shape, jnp.bfloat16, lo, hi)
    def permutation(self, n):
        return jax.random.permutation(self._next(), n)


kernel_name = 'sequential_preLN__linear_kernel_hedgehog__geglu_ffn__prompt'

def setup_inputs():
    _rng = _Rng(jax.random.key(int.from_bytes(__import__("os").urandom(4), "little")))
    _w = (lambda a: (lambda t: t.astype(jnp.bfloat16) if jnp.issubdtype(t.dtype, jnp.floating) else t)(jnp.asarray(a)))
    def _A_setup():
        B, S, D, H = 1, 2048, 640, 32
        Dh = D // H
        return {
            "x": _w((lambda *s: _rng.normal(s) * 0.05)(B, S, D)),
            "wqkv": _w((lambda *s: _rng.normal(s) * 0.2)(D, 3 * D)),
            "w_phi": _w((lambda *s: _rng.normal(s) * 0.2)(H, Dh, Dh) * (Dh ** -0.5)),
            "wo": _w((lambda *s: _rng.normal(s) * 0.05)(D, D)),
        }
    _A_in = _A_setup()

    def _B_setup():
        B, S, D, F = 1, 2048, 640, 1536
        return {
            "x": _w((lambda *s: _rng.normal(s) * 0.05)(B, S, D)),
            "w_gate": _w((lambda *s: _rng.normal(s) * 0.05)(D, F)),
            "w_up": _w((lambda *s: _rng.normal(s) * 0.05)(D, F)),
            "w_down": _w((lambda *s: _rng.normal(s) * 0.05)(F, D)),
        }
    _B_in = _B_setup()

    return {
        "A_x": _A_in["x"],
        "A_wqkv": _A_in["wqkv"],
        "A_w_phi": _A_in["w_phi"],
        "A_wo": _A_in["wo"],
        "B_x": _B_in["x"],
        "B_w_gate": _B_in["w_gate"],
        "B_w_up": _B_in["w_up"],
        "B_w_down": _B_in["w_down"],
    }

def reference(A_x, A_wqkv, A_w_phi, A_wo, B_x, B_w_gate, B_w_up, B_w_down):
    def _A_ref(x, wqkv, w_phi, wo):
        B, S, D = x.shape
        H = 32; Dh = D // H
        qkv = (lambda x, *d: x.transpose(*d))((x @ wqkv).reshape(B, S, 3, H, Dh), 2, 0, 3, 1, 4)
        q, k, v = qkv[0], qkv[1], qkv[2]
        pq = jnp.einsum("bhsd,hdf->bhsf", q, w_phi)
        pk = jnp.einsum("bhsd,hdf->bhsf", k, w_phi)
        phi_q = jnp.concatenate([_softmax(pq, axis=-1), _softmax(-pq, axis=-1)], axis=-1)
        phi_k = jnp.concatenate([_softmax(pk, axis=-1), _softmax(-pk, axis=-1)], axis=-1)
        kv = jnp.einsum("bhsf,bhsd->bhfd", phi_k, v)
        z  = jnp.einsum("bhsf->bhf", phi_k)
        num = jnp.einsum("bhqf,bhfd->bhqd", phi_q, kv)
        den = jnp.einsum("bhqf,bhf->bhq", phi_q, z)[..., None] + 1e-6
        o = num / den
        return (lambda x, *d: x.transpose(*d))(o, 0, 2, 1, 3).reshape(B, S, D) @ wo

    def _B_ref(x, w_gate, w_up, w_down):
        return (_gelu(x @ w_gate) * (x @ w_up)) @ w_down

    x = A_x
    h = x + _A_ref(_layernorm(x, axis=-1), A_wqkv, A_w_phi, A_wo)
    h2 = h + _B_ref(_layernorm(h, axis=-1), B_w_gate, B_w_up, B_w_down)
    return h2
```

```python
import functools
import jax
import jax.numpy as jnp
from jax import lax
import jax.experimental.pallas as pl
import jax.experimental.pallas.tpu as pltpu

S, D, H, DH, F = 2048, 640, 32, 20, 1536
NP = H // 2
PR = 2 * DH
PX = PR + 8
T = 256
N = S // T
FC = 512
LOG2E = 1.4426950408889634
BF = jnp.bfloat16
F32 = jnp.float32
I32 = jnp.int32

SEM_PHI, SEM_K, SEM_V, SEM_Q, SEM_O, SEM_G, SEM_U, SEM_D, SEM_X = 0, 1, 2, 3, 4, 5, 6, 7, 8


def _nt(a, b):
    return lax.dot_general(a, b, (((1,), (1,)), ((), ())), preferred_element_type=F32)


def _nn(a, b):
    return lax.dot_general(a, b, (((1,), (0,)), ((), ())), preferred_element_type=F32)


def _ln(x):
    m = jnp.mean(x, axis=-1, keepdims=True)
    xc = x - m
    v = jnp.mean(xc * xc, axis=-1, keepdims=True)
    return xc * lax.rsqrt(v + 1e-5)


def _pair_reduce(x, op):
    x = op(x, pltpu.roll(x, 2, 1))
    return op(x, pltpu.roll(x, 4, 1))


def _feat(p):
    t = p.shape[-1]
    p4 = p.reshape(NP, 5, 8, t)
    mx = _pair_reduce(jnp.max(p4, axis=1), jnp.maximum)[:, None]
    mn = _pair_reduce(jnp.min(p4, axis=1), jnp.minimum)[:, None]
    ep = jnp.exp2(p4 - mx)
    en = jnp.exp2(mn - p4)
    sp = _pair_reduce(jnp.sum(ep, axis=1), jnp.add)[:, None]
    sn = _pair_reduce(jnp.sum(en, axis=1), jnp.add)[:, None]
    ep = ep * (1.0 / sp)
    en = en * (1.0 / sn)
    return jnp.concatenate([ep, en], axis=1).reshape(NP, 2 * PR, t).astype(BF)


def _div20(d):
    return (d * 3277) >> 16


def _kernel(x_hbm, wqkv_hbm, wphi_hbm, wo_hbm, wg_hbm, wu_hbm, wd_hbm, o_ref,
            x_ref, wq_ref, wk_ref, wv_ref, wphi_ref, wo_ref, wg_ref, wu_ref, wd_ref,
            wqt_ref, wkvt_ref, xn_ref, phiq_ref, kv_ref, kvb_ref, h_ref, hn_ref, sems):
    s = pl.program_id(0)

    def cp(src, dst, k):
        return pltpu.make_async_copy(src, dst, sems.at[k])

    c_phi = cp(wphi_hbm, wphi_ref, SEM_PHI)
    c_q = cp(wqkv_hbm.at[:, 0:D], wq_ref, SEM_Q)
    c_k = cp(wqkv_hbm.at[:, D:2 * D], wk_ref, SEM_K)
    c_v = cp(wqkv_hbm.at[:, 2 * D:3 * D], wv_ref, SEM_V)
    c_o = cp(wo_hbm, wo_ref, SEM_O)
    c_g = cp(wg_hbm, wg_ref, SEM_G)
    c_u = cp(wu_hbm, wu_ref, SEM_U)
    c_d = cp(wd_hbm, wd_ref, SEM_D)

    def c_x(i):
        r = pl.ds(pl.multiple_of(i * T, T), T)
        return cp(x_hbm.at[r, :], x_ref.at[r, :], SEM_X + i)

    def x_tile(i):
        return x_ref[pl.ds(pl.multiple_of(i * T, T), T), :].astype(F32)

    def kv_part(xn, first):
        pk = _nt(wkvt_ref[0:D, :], xn)
        vt = _nt(wkvt_ref[D:2 * D, :], xn)
        phik = _feat(pk)
        vx = jnp.concatenate([vt.reshape(NP, 5, 8, T), jnp.ones((NP, 1, 8, T), F32)], axis=1)
        vx = vx.reshape(NP, PX, T).astype(BF)
        for p in range(NP):
            r = _nt(vx[p], phik[p])
            if first:
                kv_ref[p] = r
            else:
                kv_ref[p] += r

    def q_part(xn, i):
        phiq_ref[i] = _feat(_nt(wqt_ref[...], xn))

    def attn_num(j):
        phiq = phiq_ref[j]
        return [_nn(kvb_ref[p], phiq[p]) for p in range(NP)]

    def attn_o(nums):
        lo = lax.broadcasted_iota(I32, (8, T), 0) < 4
        os_ = []
        for p in range(NP):
            nm = nums[p]
            r = 1.0 / (nm[PR:PX] + 1e-6)
            rr = pltpu.roll(r, 4, 0)
            r0 = jnp.where(lo, r, rr)
            r1 = jnp.where(lo, rr, r)
            os_ += [nm[0:8] * r0, nm[8:16] * r0, nm[16:24] * r, nm[24:32] * r1, nm[32:40] * r1]
        return jnp.concatenate(os_, axis=0).T.astype(BF)

    def attn_fin(o, j):
        h = x_tile(j) + _nn(o, wo_ref[...])
        h_ref[...] = h
        hn_ref[...] = _ln(h).astype(BF)

    def ffn_gu(hn, c):
        return _nn(hn, wg_ref[:, FC * c:FC * (c + 1)]), _nn(hn, wu_ref[:, FC * c:FC * (c + 1)])

    def ffn_down(gu, c):
        a = (jax.nn.gelu(gu[0], approximate=True) * gu[1]).astype(BF)
        return _nn(a, wd_ref[FC * c:FC * (c + 1), :])

    @pl.when(s == 0)
    def _p0():
        c_phi.start(); c_x(0).start(); c_k.start(); c_v.start(); c_q.start()
        for i in range(1, N):
            c_x(i).start()
        c_o.start(); c_g.start(); c_u.start(); c_d.start()

        hh = lax.broadcasted_iota(I32, (H, D), 0)
        dd_ = lax.broadcasted_iota(I32, (H, D), 1)
        rmat = jnp.where(_div20(dd_) == hh, 1.0, 0.0).astype(BF)
        d1 = lax.broadcasted_iota(I32, (DH, D), 1)
        dmod = d1 - DH * _div20(d1)
        c_phi.wait()
        xp = jnp.zeros((DH, D), F32)
        for dd in range(DH):
            xp = jnp.where(dmod == dd, _nn(wphi_ref[dd], rmat), xp)
        r = lax.broadcasted_iota(I32, (PX, DH), 0)
        c = lax.broadcasted_iota(I32, (PX, DH), 1)
        et = jnp.where((r >> 1) == c, 1.0, 0.0).astype(BF)
        ap = _nn(et, xp.astype(BF))[0:PR]
        r = lax.broadcasted_iota(I32, (PR, 128), 0)
        c = lax.broadcasted_iota(I32, (PR, 128), 1)
        a_t = []
        for t in range(5):
            blocks = []
            hd = _div20(c + 128 * t)
            for p in range(3 * t, 3 * t + 4):
                blocks.append(jnp.where(hd == 2 * p + (r & 1), ap[:, 128 * t:128 * (t + 1)], 0.0))
            a_t.append(jnp.concatenate(blocks, axis=0).astype(BF))

        def fold(w_ref):
            res = [_nt(a_t[t], w_ref[:, 128 * t:128 * (t + 1)]) for t in range(5)]
            out = []
            for t in range(5):
                first = res[t][0:PR] if t == 0 else res[t][0:PR] + res[t - 1][3 * PR:4 * PR]
                out += [first, res[t][PR:3 * PR]]
            out.append(res[4][3 * PR:4 * PR])
            return (jnp.concatenate(out, axis=0) * LOG2E).astype(BF)

        c_x(0).wait()
        xn = _ln(x_tile(0)).astype(BF)
        xn_ref[...] = xn
        c_k.wait()
        wkvt_ref[0:D, :] = fold(wk_ref)
        c_v.wait()
        r = lax.broadcasted_iota(I32, (128, 128), 0)
        c = lax.broadcasted_iota(I32, (128, 128), 1)
        eye = jnp.where(r == c, 1.0, 0.0).astype(BF)
        for t in range(5):
            wkvt_ref[D + 128 * t:D + 128 * (t + 1), :] = _nt(eye, wv_ref[:, 128 * t:128 * (t + 1)]).astype(BF)
        c_q.wait()
        wqt_ref[...] = fold(wq_ref)
        kv_part(xn, True)

    @pl.when(jnp.logical_and(s >= 1, s < N))
    def _p1():
        c_x(s).wait()
        xn_prev = xn_ref[...]
        xn = _ln(x_tile(s)).astype(BF)
        xn_ref[...] = xn
        q_part(xn_prev, s - 1)
        kv_part(xn, False)

    @pl.when(s == N)
    def _p2():
        r = lax.broadcasted_iota(I32, (PX, 2 * PR), 0)
        c = lax.broadcasted_iota(I32, (PX, 2 * PR), 1)
        jr = jnp.where(r < PR, jnp.where(r >= DH, 1, 0), jnp.where(r >= PR + 4, 1, 0))
        same = jr == (c & 1)
        for p in range(NP):
            kvb_ref[p] = jnp.where(same, kv_ref[p], 0.0).astype(BF)
        c_o.wait()
        nums = attn_num(0)
        pq = _nt(wqt_ref[...], xn_ref[...])
        o = attn_o(nums)
        attn_fin(o, 0)
        phiq_ref[N - 1] = _feat(pq)
        c_g.wait(); c_u.wait(); c_d.wait()

    @pl.when(jnp.logical_and(s > N, s < 2 * N))
    def _p3():
        j = s - N
        hn = hn_ref[...]
        acc = h_ref[...]
        nums = attn_num(j)
        gu0 = ffn_gu(hn, 0)
        o = attn_o(nums)
        attn_fin(o, j)
        gu1 = ffn_gu(hn, 1)
        acc = acc + ffn_down(gu0, 0)
        gu2 = ffn_gu(hn, 2)
        acc = acc + ffn_down(gu1, 1)
        acc = acc + ffn_down(gu2, 2)
        o_ref[...] = acc.astype(o_ref.dtype)

    @pl.when(s == 2 * N)
    def _p4():
        hn = hn_ref[...]
        acc = h_ref[...]
        gu0 = ffn_gu(hn, 0)
        gu1 = ffn_gu(hn, 1)
        acc = acc + ffn_down(gu0, 0)
        gu2 = ffn_gu(hn, 2)
        acc = acc + ffn_down(gu1, 1)
        acc = acc + ffn_down(gu2, 2)
        o_ref[...] = acc.astype(o_ref.dtype)


@jax.jit
def pallas_sequential_preLN__linear_kernel_hedgehog__geglu_ffn__prompt_kernel(
    A_x, A_wqkv, A_w_phi, A_wo, B_x, B_w_gate, B_w_up, B_w_down,
):
    x = A_x.reshape(S, D)
    wphi = A_w_phi.transpose(1, 2, 0)
    any_spec = pl.BlockSpec(memory_space=pl.ANY)
    out = pl.pallas_call(
        _kernel,
        grid=(2 * N + 1,),
        in_specs=[any_spec] * 7,
        out_specs=pl.BlockSpec((T, D), lambda s: (jnp.maximum(s - N - 1, 0), 0)),
        out_shape=jax.ShapeDtypeStruct((S, D), BF),
        scratch_shapes=[
            pltpu.VMEM((S, D), BF),
            pltpu.VMEM((D, D), BF),
            pltpu.VMEM((D, D), BF),
            pltpu.VMEM((D, D), BF),
            pltpu.VMEM((DH, DH, H), BF),
            pltpu.VMEM((D, D), BF),
            pltpu.VMEM((D, F), BF),
            pltpu.VMEM((D, F), BF),
            pltpu.VMEM((F, D), BF),
            pltpu.VMEM((D, D), BF),
            pltpu.VMEM((2 * D, D), BF),
            pltpu.VMEM((T, D), BF),
            pltpu.VMEM((N, NP, 2 * PR, T), BF),
            pltpu.VMEM((NP, PX, 2 * PR), F32),
            pltpu.VMEM((NP, PX, 2 * PR), BF),
            pltpu.VMEM((T, D), F32),
            pltpu.VMEM((T, D), BF),
            pltpu.SemaphoreType.DMA((SEM_X + N,)),
        ],
        compiler_params=pltpu.CompilerParams(
            dimension_semantics=("arbitrary",),
            vmem_limit_bytes=100 * 1024 * 1024,
        ),
    )(x, A_wqkv, wphi, A_wo, B_w_gate, B_w_up, B_w_down)
    return out.reshape(1, S, D)
```

```python
import jax
import jax.numpy as jnp
from jax import lax
import jax.experimental.pallas as pl
import jax.experimental.pallas.tpu as pltpu

S, D, H, DH, F = 2048, 640, 32, 20, 1536
NP = H // 2
PR = 2 * DH
PX = PR + 8
T = 256
N = S // T
FC = 512
LOG2E = 1.4426950408889634
BF = jnp.bfloat16
F32 = jnp.float32
I32 = jnp.int32
OBS = (0, 128, 192, 224, 256)
KA = 3
LNB = 32
NF1 = 7
NF2 = 2
QC = 80

SEM_PHI, SEM_K, SEM_KB, SEM_V, SEM_W, SEM_X0, SEM_X2, SEM_OUT, NSEM = range(9)


def _nt(a, b):
    return lax.dot_general(a, b, (((1,), (1,)), ((), ())), preferred_element_type=F32)


def _nn(a, b):
    return lax.dot_general(a, b, (((1,), (0,)), ((), ())), preferred_element_type=F32)


def _recip(x):
    r = pl.reciprocal(x, approx=True)
    return r * (2.0 - x * r)


def _ln(x):
    m = jnp.mean(x, axis=-1, keepdims=True)
    xc = x - m
    v = jnp.mean(xc * xc, axis=-1, keepdims=True)
    return xc * lax.rsqrt(v + 1e-5)


def _tree(op, xs):
    xs = list(xs)
    while len(xs) > 1:
        xs = [op(xs[i], xs[i + 1]) if i + 1 < len(xs) else xs[i] for i in range(0, len(xs), 2)]
    return xs[0]


def _pair_reduce(op, slabs):
    x = _tree(op, slabs)
    x = op(x, pltpu.roll(x, 2, 0))
    return op(x, pltpu.roll(x, 4, 0))


def _feat(p):
    sl = [p[8 * i:8 * (i + 1)] for i in range(5)]
    mx = _pair_reduce(jnp.maximum, sl)
    mn = _pair_reduce(jnp.minimum, sl)
    ep = [jnp.exp2(v - mx) for v in sl]
    en = [jnp.exp2(mn - v) for v in sl]
    rp = _recip(_pair_reduce(jnp.add, ep))
    rn = _recip(_pair_reduce(jnp.add, en))
    return jnp.concatenate([v * rp for v in ep] + [v * rn for v in en], axis=0).astype(BF)


def _div20(d):
    return (d * 3277) >> 16


def _weave(main, side):
    done = 0
    for i, f in enumerate(main):
        f()
        upto = (len(side) * (i + 1)) // len(main)
        for g in side[done:upto]:
            g()
        done = upto


def _kernel(x_hbm, wqkv_hbm, wphi_hbm, wo_hbm, wg_hbm, wu_hbm, wd_hbm, o_hbm,
            x_ref, wq_ref, wk_ref, wv_ref, wphi_ref, wo_ref, wg_ref, wu_ref, wd_ref,
            wqt_ref, wkt_ref, wvt_ref, xn_ref, pq_ref, kv_ref, kvb_ref, h_ref, hn_ref, ob_ref, sems):

    def cp(src, dst, k):
        return pltpu.make_async_copy(src, dst, sems.at[k])

    c_phi = lambda: cp(wphi_hbm, wphi_ref, SEM_PHI)
    c_q = lambda: cp(wqkv_hbm.at[:, 0:D], wq_ref, SEM_V)
    c_k = lambda: cp(wqkv_hbm.at[:, D:D + 128 * KA], wk_ref.at[:, 0:128 * KA], SEM_K)
    c_kb = lambda: cp(wqkv_hbm.at[:, D + 128 * KA:2 * D], wk_ref.at[:, 128 * KA:D], SEM_KB)
    c_v = lambda: cp(wqkv_hbm.at[:, 2 * D:3 * D], wv_ref, SEM_V)
    c_w = lambda: [cp(wo_hbm, wo_ref, SEM_W), cp(wg_hbm, wg_ref, SEM_W),
                   cp(wu_hbm, wu_ref, SEM_W), cp(wd_hbm, wd_ref, SEM_W)]
    c_x0 = lambda: cp(x_hbm.at[0:T, :], x_ref.at[0:T, :], SEM_X0)
    c_x1 = lambda: cp(x_hbm.at[T:2 * T, :], x_ref.at[T:2 * T, :], SEM_KB)
    c_x2 = lambda: cp(x_hbm.at[2 * T:S, :], x_ref.at[2 * T:S, :], SEM_X2)

    def rows(start, n):
        return pl.ds(start, n) if isinstance(start, int) else pl.ds(pl.multiple_of(start, 16), n)

    def c_out(start, n):
        return cp(ob_ref.at[rows(start, n), :], o_hbm.at[rows(start, n), :], SEM_OUT)

    def x_tile(i):
        return x_ref[rows(i * T, T), :].astype(F32)

    def ln1_units(i):
        def unit(b):
            def f():
                xb = x_ref[rows(i * T + b * LNB, LNB), :].astype(F32)
                xn_ref[i, b * LNB:(b + 1) * LNB] = _ln(xb).astype(BF)
            return f
        return [unit(b) for b in range(T // LNB)]

    def k_feat(pk):
        return [_feat(pk[PR * p:PR * (p + 1)]) for p in range(NP)]

    def kv_acc(phik, vt, first, ps=range(NP)):
        ones = jnp.ones((8, T), F32)
        for p in ps:
            vx = jnp.concatenate([vt[PR * p:PR * (p + 1)], ones], axis=0).astype(BF)
            r = _nt(vx, phik[p])
            if first:
                kv_ref[p] = r
            else:
                kv_ref[p] += r

    def q_proj(i, lo, hi):
        pq_ref[i, lo:hi] = _nt(wqt_ref[lo:hi], xn_ref[i])

    def q_units(i, lo, hi, step=QC):
        return [(lambda a=a: q_proj(i, a, min(a + step, hi))) for a in range(lo, hi, step)]

    def kv_tile(i):
        pk = _nt(wkt_ref[...], xn_ref[i])
        vt = _nt(wvt_ref[...], xn_ref[i])
        kv_acc(k_feat(pk), vt, False)

    def attn_pair(j, p):
        nm = _nn(kvb_ref[p], _feat(pq_ref[j, PR * p:PR * (p + 1)]))
        lo = lax.broadcasted_iota(I32, (8, T), 0) < 4
        r = _recip(nm[PR:PX] + 1e-6)
        rr = pltpu.roll(r, 4, 0)
        r0 = jnp.where(lo, r, rr)
        r1 = jnp.where(lo, rr, r)
        return [nm[0:8] * r0, nm[8:16] * r0, nm[16:24] * r, nm[24:32] * r1, nm[32:40] * r1]

    def attn_fin(slabs, j):
        o = jnp.concatenate(slabs, axis=0).T.astype(BF)
        h = x_tile(j) + _nn(o, wo_ref[...])
        h_ref[...] = h
        hn_ref[...] = _ln(h).astype(BF)

    def ffn_gu(hn, c, between=None):
        if between is None:
            return _nn(hn, wg_ref[:, FC * c:FC * (c + 1)]), _nn(hn, wu_ref[:, FC * c:FC * (c + 1)])
        g, u = [], []
        for t in range(FC // 128):
            lo = FC * c + 128 * t
            g.append(_nn(hn, wg_ref[:, lo:lo + 128]))
            between(2 * t)
            u.append(_nn(hn, wu_ref[:, lo:lo + 128]))
            between(2 * t + 1)
        return jnp.concatenate(g, axis=1), jnp.concatenate(u, axis=1)

    def ffn_down(gu, c):
        a = (jax.nn.gelu(gu[0], approximate=True) * gu[1]).astype(BF)
        return _nn(a, wd_ref[FC * c:FC * (c + 1), :])

    c_phi().start(); c_x0().start(); c_k().start(); c_x1().start(); c_kb().start(); c_v().start(); c_q().start()
    c_x2().start()
    for c in c_w():
        c.start()

    hh = lax.broadcasted_iota(I32, (H, D), 0)
    dd_ = lax.broadcasted_iota(I32, (H, D), 1)
    rmat = jnp.where(_div20(dd_) == hh, 1.0, 0.0).astype(BF)
    d1 = lax.broadcasted_iota(I32, (DH, D), 1)
    dmod = d1 - DH * _div20(d1)
    c_phi().wait()
    xp = jnp.zeros((DH, D), F32)
    for dd in range(DH):
        xp = jnp.where(dmod == dd, _nn(wphi_ref[dd], rmat), xp)
    r = lax.broadcasted_iota(I32, (PX, DH), 0)
    c = lax.broadcasted_iota(I32, (PX, DH), 1)
    et = jnp.where((r >> 1) == c, 1.0, 0.0).astype(BF)
    ap = _nn(et, xp.astype(BF))[0:PR]
    r = lax.broadcasted_iota(I32, (PR, 128), 0)
    c = lax.broadcasted_iota(I32, (PR, 128), 1)
    a_t = []
    for t in range(5):
        blocks = []
        hd = _div20(c + 128 * t)
        for p in range(3 * t, 3 * t + 4):
            blocks.append(jnp.where(hd == 2 * p + (r & 1), ap[:, 128 * t:128 * (t + 1)], 0.0))
        a_t.append(jnp.concatenate(blocks, axis=0).astype(BF))

    def fold_dot(w_ref, t):
        return _nt(a_t[t], w_ref[:, 128 * t:128 * (t + 1)])

    def fold_rows(res, t):
        first = res[t][0:PR] if t == 0 else res[t][0:PR] + res[t - 1][3 * PR:4 * PR]
        return [first, res[t][PR:(3 if t < 4 else 4) * PR]]

    def fold_fin(parts):
        return (jnp.concatenate(parts, axis=0) * LOG2E).astype(BF)

    def ln1(i):
        xn_ref[i] = _ln(x_tile(i)).astype(BF)

    def proj(w_ref, i, cuts):
        return jnp.concatenate([_nt(w_ref[lo:hi], xn_ref[i]) for lo, hi in zip(cuts[:-1], cuts[1:])], axis=0)

    def feats(pk, ps, base=0):
        return [_feat(pk[PR * (p - base):PR * (p - base + 1)]) for p in ps]

    c_x0().wait()
    ln1(0)
    c_k().wait()
    res = [fold_dot(wk_ref, t) for t in range(3)]
    head = jnp.concatenate(sum([fold_rows(res, t) for t in range(3)], []), axis=0)
    wkt_ref[0:320] = fold_fin([head[0:320]])
    pk0a = proj(wkt_ref, 0, (0, 160, 240, 320))
    phik0 = feats(pk0a, range(4))
    c_x1().wait()
    c_kb().wait()
    res.append(fold_dot(wk_ref, 3))
    phik0 += feats(pk0a, range(4, 6))
    res.append(fold_dot(wk_ref, 4))
    phik0 += feats(pk0a, range(6, 8))
    wkt_ref[320:D] = fold_fin([head[320:360]] + fold_rows(res, 3) + fold_rows(res, 4))
    pk0b = proj(wkt_ref, 0, (320, D))
    ln1(1)
    pk1 = proj(wkt_ref, 1, (0, 320, 480, 560, D))
    phik0 += feats(pk0b, range(8, 16), 8)
    phik1 = feats(pk1, range(12))
    c_v().wait()
    c_q().wait()
    resq = []
    for t in range(5):
        wvt_ref[:, 128 * t:128 * (t + 1)] = wv_ref[128 * t:128 * (t + 1), :].T
        resq.append(fold_dot(wq_ref, t))
    wqt_ref[...] = fold_fin(sum([fold_rows(resq, t) for t in range(5)], []))
    vt0 = _nt(wvt_ref[...], xn_ref[0])
    vt1 = _nt(wvt_ref[...], xn_ref[1])
    kv_acc(phik0, vt0, True)
    phik1 += feats(pk1, range(12, 16))
    kv_acc(phik1, vt1, False, range(12))
    for g in range(3):
        kv_acc(phik1, vt1, False, range(12 + g, 13 + g if g < 2 else 16))
        q_proj(0, 80 * g, 80 * (g + 1))
    c_x2().wait()

    def p1(it, carry):
        t0 = 2 + 3 * it
        for k in range(3):
            q_proj(t0 - 2 + k, 240 if k == 0 else 0, D)
            ln1(t0 + k)
            kv_tile(t0 + k)
        for lo in (0, 80, 160):
            q_proj(t0 + 1, lo, lo + 80)
        return carry

    lax.fori_loop(0, 2, p1, 0)

    for c in c_w():
        c.wait()
    r = lax.broadcasted_iota(I32, (PX, 2 * PR), 0)
    c = lax.broadcasted_iota(I32, (PX, 2 * PR), 1)
    jr = jnp.where(r < PR, jnp.where(r >= DH, 1, 0), jnp.where(r >= PR + 4, 1, 0))
    same = jr == (c & 1)
    for p in range(NP):
        kvb_ref[p] = jnp.where(same, kv_ref[p], 0.0).astype(BF)
    slabs = []
    fill = [(N - 2, lo) for lo in range(240, D, 80)] + [(N - 1, lo) for lo in range(0, D, 80)]
    for g in range(8):
        if g < NF1:
            i, lo = fill.pop(0)
            q_proj(i, lo, lo + 80)
        slabs += attn_pair(0, 2 * g) + attn_pair(0, 2 * g + 1)
    for g in range(NF2):
        i, lo = fill.pop(0)
        q_proj(i, lo, lo + 80)
    attn_fin(slabs, 0)
    for i, lo in fill:
        q_proj(i, lo, lo + 80)

    def p3(j, carry):
        hn = hn_ref[...]
        acc = h_ref[...]
        slabs = []

        def between(t):
            slabs.extend(attn_pair(j, 2 * t) + attn_pair(j, 2 * t + 1))

        gu0 = ffn_gu(hn, 0, between)
        gu1 = ffn_gu(hn, 1)
        attn_fin(slabs, j)
        acc = acc + ffn_down(gu0, 0)
        gu2 = ffn_gu(hn, 2)
        acc = acc + ffn_down(gu1, 1)
        acc = acc + ffn_down(gu2, 2)
        ob_ref[rows((j - 1) * T, T), :] = acc.astype(BF)
        c_out((j - 1) * T, T).start()
        return carry

    lax.fori_loop(1, N, p3, 0)

    hn = hn_ref[...]
    acc = h_ref[...]
    gu0 = ffn_gu(hn, 0)
    gu1 = ffn_gu(hn, 1)
    acc = acc + ffn_down(gu0, 0)
    gu2 = ffn_gu(hn, 2)
    acc = acc + ffn_down(gu1, 1)
    for lo, hi in zip(OBS[:-1], OBS[1:]):
        y = acc[lo:hi] + ffn_down((gu2[0][lo:hi], gu2[1][lo:hi]), 2)
        start = (N - 1) * T + lo
        ob_ref[rows(start, hi - lo), :] = y.astype(BF)
        c_out(start, hi - lo).start()
    cp(ob_ref, o_hbm, SEM_OUT).wait()


@jax.jit
def pallas_sequential_preLN__linear_kernel_hedgehog__geglu_ffn__prompt_kernel(
    A_x, A_wqkv, A_w_phi, A_wo, B_x, B_w_gate, B_w_up, B_w_down,
):
    x = A_x.reshape(S, D)
    wphi = A_w_phi.transpose(1, 2, 0)
    any_spec = pl.BlockSpec(memory_space=pl.ANY)
    out = pl.pallas_call(
        _kernel,
        in_specs=[any_spec] * 7,
        out_specs=any_spec,
        out_shape=jax.ShapeDtypeStruct((S, D), BF),
        scratch_shapes=[
            pltpu.VMEM((S, D), BF),
            pltpu.VMEM((D, D), BF),
            pltpu.VMEM((D, D), BF),
            pltpu.VMEM((D, D), BF),
            pltpu.VMEM((DH, DH, H), BF),
            pltpu.VMEM((D, D), BF),
            pltpu.VMEM((D, F), BF),
            pltpu.VMEM((D, F), BF),
            pltpu.VMEM((F, D), BF),
            pltpu.VMEM((D, D), BF),
            pltpu.VMEM((D, D), BF),
            pltpu.VMEM((D, D), BF),
            pltpu.VMEM((N, T, D), BF),
            pltpu.VMEM((N, D, T), F32),
            pltpu.VMEM((NP, PX, 2 * PR), F32),
            pltpu.VMEM((NP, PX, 2 * PR), BF),
            pltpu.VMEM((T, D), F32),
            pltpu.VMEM((T, D), BF),
            pltpu.VMEM((S, D), BF),
            pltpu.SemaphoreType.DMA((NSEM,)),
        ],
        compiler_params=pltpu.CompilerParams(
            vmem_limit_bytes=100 * 1024 * 1024,
        ),
    )(x, A_wqkv, wphi, A_wo, B_w_gate, B_w_up, B_w_down)
    return out.reshape(1, S, D)
```

```python
import jax
import jax.numpy as jnp
from jax import lax
import jax.experimental.pallas as pl
import jax.experimental.pallas.tpu as pltpu

S, D, H, DH, F = 2048, 640, 32, 20, 1536
NP = H // 2
PR = 2 * DH
PX = PR + 8
T = 256
N = S // T
TH = 128
FC = 512
KA = 384
OBS = (0, 64, 96, 128)
LOG2E = 1.4426950408889634
BF = jnp.bfloat16
F32 = jnp.float32
I32 = jnp.int32

SEM_PHI, SEM_X0, SEM_KA, SEM_KB, SEM_QV, SEM_X2, SEM_W, SEM_OUT, NSEM = range(9)


def _nt(a, b):
    return lax.dot_general(a, b, (((1,), (1,)), ((), ())), preferred_element_type=F32)


def _nn(a, b):
    return lax.dot_general(a, b, (((1,), (0,)), ((), ())), preferred_element_type=F32)


def _recip(x):
    r = pl.reciprocal(x, approx=True)
    return r * (2.0 - x * r)


def _ln(x):
    m = jnp.mean(x, axis=-1, keepdims=True)
    xc = x - m
    v = jnp.mean(xc * xc, axis=-1, keepdims=True)
    return xc * lax.rsqrt(v + 1e-5)


def _tree(op, xs):
    xs = list(xs)
    while len(xs) > 1:
        xs = [op(xs[i], xs[i + 1]) if i + 1 < len(xs) else xs[i] for i in range(0, len(xs), 2)]
    return xs[0]


def _pair_reduce(op, slabs):
    x = _tree(op, slabs)
    x = op(x, pltpu.roll(x, 2, 0))
    return op(x, pltpu.roll(x, 4, 0))


def _feat(p):
    sl = [p[8 * i:8 * (i + 1)] for i in range(5)]
    mx = _pair_reduce(jnp.maximum, sl)
    mn = _pair_reduce(jnp.minimum, sl)
    ep = [jnp.exp2(v - mx) for v in sl]
    en = [jnp.exp2(mn - v) for v in sl]
    rp = _recip(_pair_reduce(jnp.add, ep))
    rn = _recip(_pair_reduce(jnp.add, en))
    return jnp.concatenate([v * rp for v in ep] + [v * rn for v in en], axis=0).astype(BF)


def _div20(d):
    return (d * 3277) >> 16


def _cuts(c):
    return zip(c[:-1], c[1:])


def _kernel(x_hbm, wqkv_hbm, wphi_hbm, wo_hbm, wg_hbm, wu_hbm, wd_hbm, o_hbm,
            x_ref, wq_ref, wka_ref, wkb_ref, wv_ref, wphi_ref, wo_ref, wg_ref, wu_ref, wd_ref,
            wqt_ref, wkt_ref, wvt_ref, xn_ref, pq_ref, kv_ref, kvb_ref, h_ref, hn_ref, ob_ref, sems):

    def cp(src, dst, k):
        return pltpu.make_async_copy(src, dst, sems.at[k])

    c_phi = lambda: [cp(wphi_hbm, wphi_ref, SEM_PHI)]
    c_x0 = lambda: [cp(x_hbm.at[0:T, :], x_ref.at[0:T, :], SEM_X0)]
    c_ka = lambda: [cp(wqkv_hbm.at[:, D:D + KA], wka_ref, SEM_KA)]
    c_kb = lambda: [cp(x_hbm.at[T:2 * T, :], x_ref.at[T:2 * T, :], SEM_KB),
                    cp(wqkv_hbm.at[:, D + KA:2 * D], wkb_ref, SEM_KB)]
    c_qv = lambda: [cp(wqkv_hbm.at[:, 2 * D:3 * D], wv_ref, SEM_QV),
                    cp(wqkv_hbm.at[:, 0:D], wq_ref, SEM_QV)]
    c_x2 = lambda: [cp(x_hbm.at[2 * T:S, :], x_ref.at[2 * T:S, :], SEM_X2),
                    cp(wo_hbm, wo_ref, SEM_X2)]
    c_w = lambda: [cp(wg_hbm, wg_ref, SEM_W), cp(wu_hbm, wu_ref, SEM_W), cp(wd_hbm, wd_ref, SEM_W)]

    def wait(group):
        for c in group():
            c.wait()

    def rows(start, n):
        return pl.ds(start, n) if isinstance(start, int) else pl.ds(pl.multiple_of(start, 16), n)

    def put_out(start, y):
        r = rows(start, y.shape[0])
        ob_ref[r, :] = y.astype(BF)
        cp(ob_ref.at[r, :], o_hbm.at[r, :], SEM_OUT).start()

    def x_tile(i):
        return x_ref[rows(i * T, T), :].astype(F32)

    def ln1(i):
        xn_ref[i] = _ln(x_tile(i)).astype(BF)

    def proj(w_ref, i, cuts):
        return jnp.concatenate([_nt(w_ref[lo:hi], xn_ref[i]) for lo, hi in _cuts(cuts)], axis=0)

    def q_proj(i, cuts):
        for lo, hi in _cuts(cuts):
            pq_ref[i, lo:hi] = _nt(wqt_ref[lo:hi], xn_ref[i])

    def feats(pk, ps, base=0):
        return [_feat(pk[PR * (p - base):PR * (p - base + 1)]) for p in ps]

    def kv_acc(phik, vt, first, ps=range(NP)):
        ones = jnp.ones((8, T), F32)
        for p in ps:
            vx = jnp.concatenate([vt[PR * p:PR * (p + 1)], ones], axis=0).astype(BF)
            r = _nt(vx, phik[p])
            if first:
                kv_ref[p] = r
            else:
                kv_ref[p] += r

    def attn_pair(j, p):
        nm = _nn(kvb_ref[p], _feat(pq_ref[j, PR * p:PR * (p + 1)]))
        lo = lax.broadcasted_iota(I32, (8, T), 0) < 4
        r = _recip(nm[PR:PX] + 1e-6)
        rr = pltpu.roll(r, 4, 0)
        r0 = jnp.where(lo, r, rr)
        r1 = jnp.where(lo, rr, r)
        return [nm[0:8] * r0, nm[8:16] * r0, nm[16:24] * r, nm[24:32] * r1, nm[32:40] * r1]

    def attn_fin(slabs, j):
        o = jnp.concatenate(slabs, axis=0).T.astype(BF)
        h = x_tile(j) + _nn(o, wo_ref[...])
        h_ref[...] = h
        hn_ref[...] = _ln(h).astype(BF)

    def ffn_gu(hn, c, between=None):
        if between is None:
            return _nn(hn, wg_ref[:, FC * c:FC * (c + 1)]), _nn(hn, wu_ref[:, FC * c:FC * (c + 1)])
        g, u = [], []
        for t in range(FC // 128):
            lo = FC * c + 128 * t
            g.append(_nn(hn, wg_ref[:, lo:lo + 128]))
            between(2 * t)
            u.append(_nn(hn, wu_ref[:, lo:lo + 128]))
            between(2 * t + 1)
        return jnp.concatenate(g, axis=1), jnp.concatenate(u, axis=1)

    def ffn_down(gu, c):
        a = (jax.nn.gelu(gu[0], approximate=True) * gu[1]).astype(BF)
        return _nn(a, wd_ref[FC * c:FC * (c + 1), :])

    for group in (c_phi, c_x0, c_ka, c_kb, c_qv, c_x2, c_w):
        for c in group():
            c.start()

    hh = lax.broadcasted_iota(I32, (H, D), 0)
    dd_ = lax.broadcasted_iota(I32, (H, D), 1)
    rmat = jnp.where(_div20(dd_) == hh, 1.0, 0.0).astype(BF)
    d1 = lax.broadcasted_iota(I32, (DH, D), 1)
    dmod = d1 - DH * _div20(d1)
    wait(c_phi)
    xp = jnp.zeros((DH, D), F32)
    for dd in range(DH):
        xp = jnp.where(dmod == dd, _nn(wphi_ref[dd], rmat), xp)
    r = lax.broadcasted_iota(I32, (PX, DH), 0)
    c = lax.broadcasted_iota(I32, (PX, DH), 1)
    et = jnp.where((r >> 1) == c, 1.0, 0.0).astype(BF)
    ap = _nn(et, xp.astype(BF))[0:PR]
    r = lax.broadcasted_iota(I32, (PR, 128), 0)
    c = lax.broadcasted_iota(I32, (PR, 128), 1)
    a_t = []
    for t in range(5):
        hd = _div20(c + 128 * t)
        a_t.append(jnp.concatenate(
            [jnp.where(hd == 2 * p + (r & 1), ap[:, 128 * t:128 * (t + 1)], 0.0)
             for p in range(3 * t, 3 * t + 4)], axis=0).astype(BF))

    def fold_rows(res, t):
        first = res[t][0:PR] if t == 0 else res[t][0:PR] + res[t - 1][3 * PR:4 * PR]
        return [first, res[t][PR:(3 if t < 4 else 4) * PR]]

    def fold_fin(parts):
        return (jnp.concatenate(parts, axis=0) * LOG2E).astype(BF)

    wait(c_x0)
    ln1(0)
    wait(c_ka)
    res = [_nt(a_t[t], wka_ref[:, 128 * t:128 * (t + 1)]) for t in range(3)]
    head = jnp.concatenate(sum([fold_rows(res, t) for t in range(3)], []), axis=0)
    wkt_ref[0:320] = fold_fin([head[0:320]])
    pk0a = proj(wkt_ref, 0, (0, 160, 240, 320))
    phik0 = feats(pk0a, range(4))

    wait(c_kb)
    res.append(_nt(a_t[3], wkb_ref[:, 0:128]))
    phik0 += feats(pk0a, range(4, 6))
    res.append(_nt(a_t[4], wkb_ref[:, 128:256]))
    phik0 += feats(pk0a, range(6, 8))
    wkt_ref[320:D] = fold_fin([head[320:360]] + fold_rows(res, 3) + fold_rows(res, 4))
    pk0b = proj(wkt_ref, 0, (320, D))
    ln1(1)
    pk1 = proj(wkt_ref, 1, (0, 320, 480, 560, D))
    phik0 += feats(pk0b, range(8, 16), 8)
    phik1 = feats(pk1, range(12))

    wait(c_qv)
    res = []
    for t in range(5):
        wvt_ref[:, 128 * t:128 * (t + 1)] = wv_ref[128 * t:128 * (t + 1), :].T
        res.append(_nt(a_t[t], wq_ref[:, 128 * t:128 * (t + 1)]))
    wqt_ref[...] = fold_fin(sum([fold_rows(res, t) for t in range(5)], []))
    vt0 = proj(wvt_ref, 0, (0, D))
    vt1 = proj(wvt_ref, 1, (0, D))
    kv_acc(phik0, vt0, True)
    phik1 += feats(pk1, range(12, 16))
    kv_acc(phik1, vt1, False, range(12))
    for g in range(3):
        kv_acc(phik1, vt1, False, range(12 + g, 13 + g if g < 2 else 16))
        q_proj(0, (80 * g, 80 * (g + 1)))

    wait(c_x2)
    for t in range(2, N):
        q_proj(t - 2, (240, D) if t == 2 else (0, 320, D))
        ln1(t)
        pk = proj(wkt_ref, t, (0, D))
        vt = proj(wvt_ref, t, (0, D))
        kv_acc(feats(pk, range(NP)), vt, False)

    r = lax.broadcasted_iota(I32, (PX, 2 * PR), 0)
    c = lax.broadcasted_iota(I32, (PX, 2 * PR), 1)
    jr = jnp.where(r < PR, jnp.where(r >= DH, 1, 0), jnp.where(r >= PR + 4, 1, 0))
    same = jr == (c & 1)
    for p in range(NP):
        kvb_ref[p] = jnp.where(same, kv_ref[p], 0.0).astype(BF)
    slabs = []
    for g in range(8):
        q_proj(N - 2, (80 * g, 80 * (g + 1)))
        slabs += attn_pair(0, 2 * g) + attn_pair(0, 2 * g + 1)
    q_proj(N - 1, (0, 240))
    attn_fin(slabs, 0)
    q_proj(N - 1, (240, 400, 480, 560, D))

    wait(c_w)

    def step(j, carry):
        hn = hn_ref[...]
        acc = h_ref[...]
        slabs = []

        def between(t):
            slabs.extend(attn_pair(j, 2 * t) + attn_pair(j, 2 * t + 1))

        gu0 = ffn_gu(hn, 0, between)
        gu1 = ffn_gu(hn, 1)
        attn_fin(slabs, j)
        acc = acc + ffn_down(gu0, 0)
        gu2 = ffn_gu(hn, 2)
        acc = acc + ffn_down(gu1, 1)
        acc = acc + ffn_down(gu2, 2)
        put_out((j - 1) * T, acc)
        return carry

    lax.fori_loop(1, N, step, 0)

    def last(u, carry):
        hn = hn_ref[rows(u * TH, TH), :]
        acc = h_ref[rows(u * TH, TH), :]
        gu0 = ffn_gu(hn, 0)
        gu1 = ffn_gu(hn, 1)
        acc = acc + ffn_down(gu0, 0)
        gu2 = ffn_gu(hn, 2)
        acc = acc + ffn_down(gu1, 1)
        for lo, hi in _cuts(OBS):
            y = acc[lo:hi] + ffn_down((gu2[0][lo:hi], gu2[1][lo:hi]), 2)
            put_out((N - 1) * T + u * TH + lo, y)
        return carry

    lax.fori_loop(0, T // TH, last, 0)
    cp(ob_ref, o_hbm, SEM_OUT).wait()


@jax.jit
def pallas_sequential_preLN__linear_kernel_hedgehog__geglu_ffn__prompt_kernel(
    A_x, A_wqkv, A_w_phi, A_wo, B_x, B_w_gate, B_w_up, B_w_down,
):
    x = A_x.reshape(S, D)
    wphi = A_w_phi.transpose(1, 2, 0)
    any_spec = pl.BlockSpec(memory_space=pl.ANY)
    out = pl.pallas_call(
        _kernel,
        in_specs=[any_spec] * 7,
        out_specs=any_spec,
        out_shape=jax.ShapeDtypeStruct((S, D), BF),
        scratch_shapes=[
            pltpu.VMEM((S, D), BF),
            pltpu.VMEM((D, D), BF),
            pltpu.VMEM((D, KA), BF),
            pltpu.VMEM((D, D - KA), BF),
            pltpu.VMEM((D, D), BF),
            pltpu.VMEM((DH, DH, H), BF),
            pltpu.VMEM((D, D), BF),
            pltpu.VMEM((D, F), BF),
            pltpu.VMEM((D, F), BF),
            pltpu.VMEM((F, D), BF),
            pltpu.VMEM((D, D), BF),
            pltpu.VMEM((D, D), BF),
            pltpu.VMEM((D, D), BF),
            pltpu.VMEM((N, T, D), BF),
            pltpu.VMEM((N, D, T), F32),
            pltpu.VMEM((NP, PX, 2 * PR), F32),
            pltpu.VMEM((NP, PX, 2 * PR), BF),
            pltpu.VMEM((T, D), F32),
            pltpu.VMEM((T, D), BF),
            pltpu.VMEM((S, D), BF),
            pltpu.SemaphoreType.DMA((NSEM,)),
        ],
        compiler_params=pltpu.CompilerParams(
            vmem_limit_bytes=100 * 1024 * 1024,
            disable_bounds_checks=True,
        ),
    )(x, A_wqkv, wphi, A_wo, B_w_gate, B_w_up, B_w_down)
    return out.reshape(1, S, D)
```

```python
import jax
import jax.numpy as jnp
from jax import lax
import jax.experimental.pallas as pl
import jax.experimental.pallas.tpu as pltpu

S, D, H, DH, F = 2048, 640, 32, 20, 1536
NP = H // 2
PR = 2 * DH
PX = PR + 8
QR = 152
DP = 4 * QR
T = 256
N = S // T
TH = 128
FC = 512
KA = 384
OBS = (0, 64, 96, 128)
Q_CUTS = {2: (304, 512, 608), 3: (0, 336, 608), 4: (0, 320, 608), 5: (0, 304, 608), 6: (0, 608), 7: (0, 192, 608)}
K_CUTS = {2: (0, 608), 3: (0, 608), 4: (0, 608), 5: (0, 240, 608), 6: (0, 192, 608), 7: (0, 608)}
V_CUTS = {2: (0, 640), 3: (0, 640), 4: (0, 352, 640), 5: (0, 640), 6: (0, 640), 7: (0, 272, 640)}
LOG2E = 1.4426950408889634
BF = jnp.bfloat16
F32 = jnp.float32
I32 = jnp.int32

SEM_PHI, SEM_X0, SEM_KA, SEM_KB, SEM_QV, SEM_X2, SEM_W, SEM_OUT, NSEM = range(9)


def _nt(a, b):
    return lax.dot_general(a, b, (((1,), (1,)), ((), ())), preferred_element_type=F32)


def _nn(a, b):
    return lax.dot_general(a, b, (((1,), (0,)), ((), ())), preferred_element_type=F32)


def _recip(x):
    r = pl.reciprocal(x, approx=True)
    return r * (2.0 - x * r)


def _ln(x):
    m = jnp.mean(x, axis=-1, keepdims=True)
    xc = x - m
    v = jnp.mean(xc * xc, axis=-1, keepdims=True)
    return xc * lax.rsqrt(v + 1e-5)


def _tree(op, xs):
    xs = list(xs)
    while len(xs) > 1:
        xs = [op(xs[i], xs[i + 1]) if i + 1 < len(xs) else xs[i] for i in range(0, len(xs), 2)]
    return xs[0]


def _pair_reduce(op, slabs):
    x = _tree(op, slabs)
    x = op(x, pltpu.roll(x, 2, 0))
    return op(x, pltpu.roll(x, 4, 0))


def _slot_is(k, t):
    return (lax.broadcasted_iota(I32, (8, t), 0) >> 1) == k


def _feat(get, p):
    q, base = p % 4, QR * (p // 4)
    sl = [get(base + 24 + 32 * q + 8 * i, base + 32 + 32 * q + 8 * i) for i in range(4)]
    t = sl[0].shape[-1]
    last = 0.0
    for m in range(3):
        last = jnp.where(_slot_is((q + m) % 4, t), get(base + 8 * m, base + 8 * (m + 1)), last)
    sl.append(last)
    mx = _pair_reduce(jnp.maximum, sl)
    mn = _pair_reduce(jnp.minimum, sl)
    ep = [jnp.exp2(v - mx) for v in sl]
    en = [jnp.exp2(mn - v) for v in sl]
    rp = _recip(_pair_reduce(jnp.add, ep))
    rn = _recip(_pair_reduce(jnp.add, en))
    return jnp.concatenate([v * rp for v in ep] + [v * rn for v in en], axis=0).astype(BF)


def _div20(d):
    return (d * 3277) >> 16


def _cuts(c):
    return zip(c[:-1], c[1:])


def _kernel(x_hbm, wqkv_hbm, wphi_hbm, wo_hbm, wg_hbm, wu_hbm, wd_hbm, o_hbm,
            x_ref, wqa_ref, wqb_ref, wka_ref, wkb_ref, wv_ref, wphi_ref, wo_ref, wg_ref, wu_ref, wd_ref,
            wqt_ref, wkt_ref, wvt_ref, xn_ref, pq_ref, kv_ref, kvb_ref, h_ref, hn_ref, ob_ref, sems):

    def cp(src, dst, k):
        return pltpu.make_async_copy(src, dst, sems.at[k])

    c_phi = lambda: [cp(wphi_hbm, wphi_ref, SEM_PHI)]
    c_x0 = lambda: [cp(x_hbm.at[0:T, :], x_ref.at[0:T, :], SEM_X0)]
    c_ka = lambda: [cp(wqkv_hbm.at[:, D:D + KA], wka_ref, SEM_KA)]
    c_kb = lambda: [cp(x_hbm.at[T:2 * T, :], x_ref.at[T:2 * T, :], SEM_KB),
                    cp(wqkv_hbm.at[:, D + KA:2 * D], wkb_ref, SEM_KB)]
    c_qv = lambda: [cp(wqkv_hbm.at[:, 2 * D:3 * D], wv_ref, SEM_QV),
                    cp(wqkv_hbm.at[:, 0:KA], wqa_ref, SEM_QV)]
    c_x2 = lambda: [cp(wqkv_hbm.at[:, KA:D], wqb_ref, SEM_X2),
                    cp(x_hbm.at[2 * T:S, :], x_ref.at[2 * T:S, :], SEM_X2),
                    cp(wo_hbm, wo_ref, SEM_X2)]
    c_w = lambda: [cp(wg_hbm, wg_ref, SEM_W), cp(wu_hbm, wu_ref, SEM_W), cp(wd_hbm, wd_ref, SEM_W)]

    def wait(group):
        for c in group():
            c.wait()

    def rows(start, n):
        return pl.ds(start, n) if isinstance(start, int) else pl.ds(pl.multiple_of(start, 16), n)

    def put_out(start, y):
        r = rows(start, y.shape[0])
        ob_ref[r, :] = y.astype(BF)
        cp(ob_ref.at[r, :], o_hbm.at[r, :], SEM_OUT).start()

    def x_tile(i):
        return x_ref[rows(i * T, T), :].astype(F32)

    def ln1(i):
        x1 = jnp.concatenate([x_ref[rows(i * T, T), 128 * t:128 * (t + 1)].astype(F32)
                              for t in range(5)], axis=1)
        xc = x_tile(i) - jnp.mean(x1, axis=-1, keepdims=True)
        v = jnp.mean(xc * xc, axis=-1, keepdims=True)
        xn_ref[i] = (xc * lax.rsqrt(v + 1e-5)).astype(BF)

    def proj(w_ref, i, cuts):
        return jnp.concatenate([_nt(w_ref[lo:hi], xn_ref[i]) for lo, hi in _cuts(cuts)], axis=0)

    def q_proj(i, cuts):
        for lo, hi in _cuts(cuts):
            pq_ref[i, lo:hi] = _nt(wqt_ref[lo:hi], xn_ref[i])

    def feats(pk, ps, base=0):
        return [_feat(lambda lo, hi: pk[lo - base:hi - base], p) for p in ps]

    def kv_acc(phik, vt, first, ps=range(NP)):
        ones = jnp.ones((8, T), F32)
        for p in ps:
            vx = jnp.concatenate([vt[PR * p:PR * (p + 1)], ones], axis=0).astype(BF)
            r = _nt(vx, phik[p])
            if first:
                kv_ref[p] = r
            else:
                kv_ref[p] += r

    def attn_pair(j, p, phiq=None):
        if phiq is None:
            phiq = _feat(lambda lo, hi: pq_ref[j, lo:hi], p)
        nm = _nn(kvb_ref[p], phiq)
        lo = lax.broadcasted_iota(I32, (8, T), 0) < 4
        r = _recip(nm[PR:PX] + 1e-6)
        rr = pltpu.roll(r, 4, 0)
        r0 = jnp.where(lo, r, rr)
        r1 = jnp.where(lo, rr, r)
        return [nm[0:8] * r0, nm[8:16] * r0, nm[16:24] * r, nm[24:32] * r1, nm[32:40] * r1]

    def attn_fin(slabs, j):
        o = jnp.concatenate(slabs, axis=0).T.astype(BF)
        h = x_tile(j) + _nn(o, wo_ref[...])
        h_ref[...] = h
        hn_ref[...] = _ln(h).astype(BF)

    def ffn_gu(hn, c, between=None):
        if between is None:
            return _nn(hn, wg_ref[:, FC * c:FC * (c + 1)]), _nn(hn, wu_ref[:, FC * c:FC * (c + 1)])
        g, u = [], []
        for t in range(FC // 128):
            lo = FC * c + 128 * t
            g.append(_nn(hn, wg_ref[:, lo:lo + 128]))
            between(2 * t)
            u.append(_nn(hn, wu_ref[:, lo:lo + 128]))
            between(2 * t + 1)
        return jnp.concatenate(g, axis=1), jnp.concatenate(u, axis=1)

    def ffn_down(gu, c):
        a = (jax.nn.gelu(gu[0], approximate=True) * gu[1]).astype(BF)
        return _nn(a, wd_ref[FC * c:FC * (c + 1), :])

    for group in (c_phi, c_x0, c_ka, c_kb, c_qv, c_x2, c_w):
        for c in group():
            c.start()

    hh = lax.broadcasted_iota(I32, (H, D), 0)
    dd_ = lax.broadcasted_iota(I32, (H, D), 1)
    rmat = jnp.where(_div20(dd_) == hh, 1.0, 0.0).astype(BF)
    d1 = lax.broadcasted_iota(I32, (DH, D), 1)
    dmod = d1 - DH * _div20(d1)
    wait(c_phi)
    xp = jnp.zeros((DH, D), F32)
    for dd in range(DH):
        xp = jnp.where(dmod == dd, _nn(wphi_ref[dd], rmat), xp)
    r = lax.broadcasted_iota(I32, (PX, DH), 0)
    c = lax.broadcasted_iota(I32, (PX, DH), 1)
    et = jnp.where((r >> 1) == c, 1.0, 0.0).astype(BF)
    ap = _nn(et, xp.astype(BF))[0:PR]
    r = lax.broadcasted_iota(I32, (PR, 128), 0)
    c = lax.broadcasted_iota(I32, (PR, 128), 1)
    a_t = []
    for t in range(5):
        hd = _div20(c + 128 * t)
        blk = ap[:, 128 * t:128 * (t + 1)]
        var = [blk] + [jnp.concatenate([blk[0:32], pltpu.roll(blk[32:40], 2 * q, 0)], axis=0)
                       for q in range(1, 4)]
        a_t.append(jnp.concatenate(
            [jnp.where(hd == 2 * p + (r & 1), var[p % 4], 0.0)
             for p in range(3 * t, 3 * t + 4)], axis=0).astype(BF))

    def fold_pair(res, p):
        t, k = (p // 3, p % 3) if p < 15 else (4, 3)
        w = res[t][PR * k:PR * (k + 1)]
        if k == 0 and t > 0:
            w = w + res[t - 1][3 * PR:4 * PR]
        ref = jnp.where(_slot_is((p + 3) % 4, D), w[32:40], 0.0)
        ref = ref + pltpu.roll(ref, 2, 0)
        ref = ref + pltpu.roll(ref, 4, 0)
        return [w[8 * i:8 * (i + 1)] - ref for i in range(5)]

    def fold_quads(res, quads):
        out = []
        for g in quads:
            ws = [fold_pair(res, 4 * g + q) for q in range(4)]
            for m in range(3):
                lm = ws[(0 - m) % 4][4]
                for s in range(1, 4):
                    lm = jnp.where(_slot_is(s, D), ws[(s - m) % 4][4], lm)
                out.append(lm)
            for q in range(4):
                out += ws[q][0:4]
        return (jnp.concatenate(out, axis=0) * LOG2E).astype(BF)

    wait(c_x0)
    ln1(0)
    wait(c_ka)
    res = [_nt(a_t[t], wka_ref[:, 128 * t:128 * (t + 1)]) for t in range(3)]
    wkt_ref[0:2 * QR] = fold_quads(res, (0, 1))
    pk0a1 = proj(wkt_ref, 0, (0, 128, 192))

    wait(c_kb)
    res += [_nt(a_t[3], wkb_ref[:, 0:128]), _nt(a_t[4], wkb_ref[:, 128:256])]
    pk0a2 = proj(wkt_ref, 0, (192, 2 * QR))
    wkt_ref[2 * QR:DP] = fold_quads(res, (2, 3))
    pk0b = proj(wkt_ref, 0, (304, 608))
    ln1(1)
    pk1 = proj(wkt_ref, 1, (0, 224, 352, 448, 528, 608))
    pk0a = jnp.concatenate([pk0a1, pk0a2], axis=0)
    phik0b = feats(pk0b, range(8, 16), 2 * QR)
    phik1 = feats(pk1, range(12))

    wait(c_qv)
    res = []
    for t in range(5):
        wvt_ref[:, 128 * t:128 * (t + 1)] = wv_ref[128 * t:128 * (t + 1), :].T
        if t < 3:
            res.append(_nt(a_t[t], wqa_ref[:, 128 * t:128 * (t + 1)]))
    wqt_ref[0:2 * QR] = fold_quads(res, (0, 1))
    q_proj(1, (0, 80))
    vt0 = proj(wvt_ref, 0, (0, 640))
    vt1 = proj(wvt_ref, 1, (0, 640))
    kv_acc(feats(pk0a, range(8)) + phik0b, vt0, True,
           (0, 1, 2, 3, 8, 9, 4, 10, 11, 5, 12, 13, 6, 14, 15, 7))
    phik1 += feats(pk1, range(12, 16))
    kv_acc(phik1, vt1, False, range(12))
    for g in range(3):
        kv_acc(phik1, vt1, False, range(12 + g, 13 + g if g < 2 else 16))
        q_proj(1, (80, 160, 240, 304)[g:g + 2])

    wait(c_x2)
    res += [_nt(a_t[3], wqb_ref[:, 0:128]), _nt(a_t[4], wqb_ref[:, 128:256])]
    wqt_ref[2 * QR:DP] = fold_quads(res, (2, 3))
    for t in range(2, N):
        q_proj(t - 1, Q_CUTS[t])
        ln1(t)
        pk = proj(wkt_ref, t, K_CUTS[t])
        vt = proj(wvt_ref, t, V_CUTS[t])
        kv_acc(feats(pk, range(NP)), vt, False)

    r = lax.broadcasted_iota(I32, (PX, 2 * PR), 0)
    c = lax.broadcasted_iota(I32, (PX, 2 * PR), 1)
    jr = jnp.where(r < PR, jnp.where(r >= DH, 1, 0), jnp.where(r >= PR + 4, 1, 0))
    same = jr == (c & 1)
    for p in range(NP):
        kvb_ref[p] = jnp.where(same, kv_ref[p], 0.0).astype(BF)
    slabs = []
    phiq0 = feats(proj(wqt_ref, 0, (0, 304, 608)), range(NP))
    for p in range(8):
        slabs += attn_pair(0, p, phiq0[p])
    q_proj(N - 1, (0, 96))
    for p in range(8, NP):
        slabs += attn_pair(0, p, phiq0[p])
    q_proj(N - 1, (96, 192))
    attn_fin(slabs, 0)
    q_proj(N - 1, (192, 336, 416, 512, 608))

    wait(c_w)

    def step(j, carry):
        hn = hn_ref[...]
        acc = h_ref[...]
        slabs = []

        def between(t):
            slabs.extend(attn_pair(j, 2 * t) + attn_pair(j, 2 * t + 1))

        gu0 = ffn_gu(hn, 0, between)
        gu1 = ffn_gu(hn, 1)
        attn_fin(slabs, j)
        acc = acc + ffn_down(gu0, 0)
        gu2 = ffn_gu(hn, 2)
        acc = acc + ffn_down(gu1, 1)
        acc = acc + ffn_down(gu2, 2)
        put_out((j - 1) * T, acc)
        return carry

    lax.fori_loop(1, N, step, 0)

    def last(u, carry):
        hn = hn_ref[rows(u * TH, TH), :]
        acc = h_ref[rows(u * TH, TH), :]
        gu0 = ffn_gu(hn, 0)
        gu1 = ffn_gu(hn, 1)
        acc = acc + ffn_down(gu0, 0)
        gu2 = ffn_gu(hn, 2)
        acc = acc + ffn_down(gu1, 1)
        for lo, hi in _cuts(OBS):
            y = acc[lo:hi] + ffn_down((gu2[0][lo:hi], gu2[1][lo:hi]), 2)
            put_out((N - 1) * T + u * TH + lo, y)
        return carry

    lax.fori_loop(0, T // TH, last, 0)
    cp(ob_ref, o_hbm, SEM_OUT).wait()


def _compiler_params():
    kw = dict(vmem_limit_bytes=100 * 1024 * 1024, disable_bounds_checks=True)
    try:
        return pltpu.CompilerParams(disable_semaphore_checks=True, **kw)
    except TypeError:
        return pltpu.CompilerParams(**kw)


@jax.jit
def pallas_sequential_preLN__linear_kernel_hedgehog__geglu_ffn__prompt_kernel(
    A_x, A_wqkv, A_w_phi, A_wo, B_x, B_w_gate, B_w_up, B_w_down,
):
    x = A_x.reshape(S, D)
    wphi = A_w_phi.transpose(1, 2, 0)
    any_spec = pl.BlockSpec(memory_space=pl.ANY)
    out = pl.pallas_call(
        _kernel,
        in_specs=[any_spec] * 7,
        out_specs=any_spec,
        out_shape=jax.ShapeDtypeStruct((S, D), BF),
        scratch_shapes=[
            pltpu.VMEM((S, D), BF),
            pltpu.VMEM((D, KA), BF),
            pltpu.VMEM((D, D - KA), BF),
            pltpu.VMEM((D, KA), BF),
            pltpu.VMEM((D, D - KA), BF),
            pltpu.VMEM((D, D), BF),
            pltpu.VMEM((DH, DH, H), BF),
            pltpu.VMEM((D, D), BF),
            pltpu.VMEM((D, F), BF),
            pltpu.VMEM((D, F), BF),
            pltpu.VMEM((F, D), BF),
            pltpu.VMEM((DP, D), BF),
            pltpu.VMEM((DP, D), BF),
            pltpu.VMEM((D, D), BF),
            pltpu.VMEM((N, T, D), BF),
            pltpu.VMEM((N, DP, T), F32),
            pltpu.VMEM((NP, PX, 2 * PR), F32),
            pltpu.VMEM((NP, PX, 2 * PR), BF),
            pltpu.VMEM((T, D), F32),
            pltpu.VMEM((T, D), BF),
            pltpu.VMEM((S, D), BF),
            pltpu.SemaphoreType.DMA((NSEM,)),
        ],
        compiler_params=_compiler_params(),
    )(x, A_wqkv, wphi, A_wo, B_w_gate, B_w_up, B_w_down)
    return out.reshape(1, S, D)
```
